```python
import os as _os
_os.environ.setdefault("JAX_PLATFORMS", "cpu")
import jax
import jax.numpy as jnp

def _softmax(x, axis=-1):
    return jax.nn.softmax(x, axis=axis)
def _gelu(x):
    return jax.nn.gelu(x, approximate=True)
def _silu(x):
    return jax.nn.silu(x)
def _sigmoid(x):
    return jax.nn.sigmoid(x)
def _layernorm(x, axis=-1, eps=1e-5):
    m = jnp.mean(x, axis=axis, keepdims=True)
    v = jnp.var(x, axis=axis, keepdims=True)
    return (x - m) / jnp.sqrt(v + eps)
def _scatter_add(tgt, idx, src, axis=0):
    return tgt.at[idx].add(src)
def _segment_sum(src, seg, n):
    return jax.ops.segment_sum(src, seg, n)
class _Rng:
    def __init__(self, key):
        self._k = key
    def _next(self):
        self._k, sub = jax.random.split(self._k)
        return sub
    def normal(self, shape):
        return jax.random.normal(self._next(), shape, dtype=jnp.bfloat16)
    def randint(self, lo, hi, shape):
        return jax.random.randint(self._next(), shape, lo, hi, dtype=jnp.int32)
    def uniform(self, shape, lo=0.0, hi=1.0):
        return jax.random.uniform(self._next(), shape, jnp.bfloat16, lo, hi)
    def permutation(self, n):
        return jax.random.permutation(self._next(), n)


kernel_name = 'concat_heads__mha_block_cached__gqa_block_cached__near_ridge'

def setup_inputs():
    _rng = _Rng(jax.random.key(int.from_bytes(__import__("os").urandom(4), "little")))
    _w = (lambda a: (lambda t: t.astype(jnp.bfloat16) if jnp.issubdtype(t.dtype, jnp.floating) else t)(jnp.asarray(a)))
    def _A_setup():
        B, Sq, D = 8, 128, 512
        H, Sk, Dh = 32, 1024, 128
        return {
            "x": _w((lambda *s: _rng.normal(s) * 0.8)(B, Sq, D)),
            "k_cache": _w((lambda *s: _rng.normal(s) * 0.8)(B, H, Sk, Dh)),
            "v_cache": _w((lambda *s: _rng.normal(s) * 0.05)(B, H, Sk, Dh)),
            "wq": _w((lambda *s: _rng.normal(s) * 0.8)(D, H * Dh) * (D ** -0.5)),
            "wo": _w((lambda *s: _rng.normal(s) * 0.05)(H * Dh, D) * ((H * Dh) ** -0.5)),
        }
    _A_in = _A_setup()

    def _B_setup():
        B, Sq, D = 8, 128, 512
        Hq, Hkv, Sk, Dh = 32, 32, 1024, 128
        assert Hq % Hkv == 0, (Hq, Hkv)
        return {
            "x": _w((lambda *s: _rng.normal(s) * 0.8)(B, Sq, D)),
            "k_cache": _w((lambda *s: _rng.normal(s) * 0.8)(B, Hkv, Sk, Dh)),
            "v_cache": _w((lambda *s: _rng.normal(s) * 0.05)(B, Hkv, Sk, Dh)),
            "wq": _w((lambda *s: _rng.normal(s) * 0.8)(D, Hq * Dh) * (D ** -0.5)),
            "wo": _w((lambda *s: _rng.normal(s) * 0.05)(Hq * Dh, D) * ((Hq * Dh) ** -0.5)),
        }
    _B_in = _B_setup()

    return {
        "A_x": _A_in["x"],
        "A_k_cache": _A_in["k_cache"],
        "A_v_cache": _A_in["v_cache"],
        "A_wq": _A_in["wq"],
        "A_wo": _A_in["wo"],
        "B_x": _B_in["x"],
        "B_k_cache": _B_in["k_cache"],
        "B_v_cache": _B_in["v_cache"],
        "B_wq": _B_in["wq"],
        "B_wo": _B_in["wo"],
    }

def reference(A_x, A_k_cache, A_v_cache, A_wq, A_wo, B_x, B_k_cache, B_v_cache, B_wq, B_wo):
    def _A_ref(x, k_cache, v_cache, wq, wo):
        B, Sq, D = x.shape
        H, Dh = 32, 128
        q = (lambda x, *d: x.transpose(*d))((x @ wq).reshape(B, Sq, H, Dh), 0, 2, 1, 3)
        scores = jnp.einsum("bhqd,bhkd->bhqk", q, k_cache) * (Dh ** -0.5)
        p = _softmax(scores, axis=-1)
        o = jnp.einsum("bhqk,bhkd->bhqd", p, v_cache)
        return (lambda x, *d: x.transpose(*d))(o, 0, 2, 1, 3).reshape(B, Sq, H * Dh) @ wo

    def _B_ref(x, k_cache, v_cache, wq, wo):
        B, Sq, D = x.shape
        Hq, Dh = 32, 128
        Hkv = k_cache.shape[1]
        rep = Hq // Hkv
        q = (lambda x, *d: x.transpose(*d))((x @ wq).reshape(B, Sq, Hq, Dh), 0, 2, 1, 3)
        k = jnp.repeat(k_cache, rep, axis=1)
        v = jnp.repeat(v_cache, rep, axis=1)
        scores = jnp.einsum("bhqd,bhkd->bhqk", q, k) * (Dh ** -0.5)
        p = _softmax(scores, axis=-1)
        o = jnp.einsum("bhqk,bhkd->bhqd", p, v)
        return (lambda x, *d: x.transpose(*d))(o, 0, 2, 1, 3).reshape(B, Sq, Hq * Dh) @ wo

    a = _A_ref(A_x, A_k_cache, A_v_cache, A_wq, A_wo)
    b = _B_ref(B_x, B_k_cache, B_v_cache, B_wq, B_wo)
    return jnp.concatenate([a, b], axis=-1)
```

```python
import jax
import jax.numpy as jnp
from jax import lax
from jax.experimental import pallas as pl
from jax.experimental.pallas import tpu as pltpu

_LOG2E = 1.4426950408889634

_R = 128
_NSLOT = 6
_DIST = 3
_NPARTS = 2


@jax.jit
def pallas_concat_heads__mha_block_cached__gqa_block_cached__near_ridge_kernel(
    A_x: jax.Array,
    A_k_cache: jax.Array,
    A_v_cache: jax.Array,
    A_wq: jax.Array,
    A_wo: jax.Array,
    B_x: jax.Array,
    B_k_cache: jax.Array,
    B_v_cache: jax.Array,
    B_wq: jax.Array,
    B_wo: jax.Array,
):
    B, Sq, D = A_x.shape
    _, H, Sk, Dh = A_k_cache.shape
    assert B_k_cache.shape == A_k_cache.shape
    assert (B, Sq, D, H, Sk, Dh) == (8, 128, 512, 32, 1024, 128)
    R, nslot, dist, nparts = _R, _NSLOT, _DIST, _NPARTS
    NP = B * H
    nch = Sk // R
    hc = nch // 2
    hstride = H // 2
    qscale = Dh ** -0.5 * _LOG2E

    def bh(j):
        b = j // H
        t = j % H
        return b, (t % 2) * hstride + t // 2

    def kern(ax, ak, av, awq, awo, bx, bk, bv, bwq, bwo, o_hbm,
             xbuf, wqbuf, wobuf, kvbuf, acc, obuf, sem_w, sem_kv, sem_o):
        kv_src = (ak, av, bk, bv)

        def chunk_copy(j, c, a):
            b, h = bh(j)
            slot = j % nslot
            return pltpu.make_async_copy(
                kv_src[a].at[b, h, pl.ds(c * R, R)],
                kvbuf.at[slot, a, pl.ds(c * R, R)],
                sem_kv.at[slot])

        unit = [(dj, cc, a) for c in range(hc)
                for dj, cc in ((0, hc + c), (1, c)) for a in range(4)]

        def issue_unit(j, part=None, only=None):
            lst = unit
            if part is not None:
                per = len(lst) // nparts
                lst = lst[part * per:(part + 1) * per]
            for dj, c, a in lst:
                if only is None or dj == only:
                    chunk_copy(j + dj, c, a).start(priority=a % 2)

        def wait_kv(j):
            slot = j % nslot
            pltpu.make_async_copy(kvbuf.at[slot], kvbuf.at[slot], sem_kv.at[slot]).wait()

        def xloop(b, c):
            for r in range(4):
                pltpu.make_async_copy(ax.at[b, pl.ds(r * 32, 32)], xbuf.at[0, b, pl.ds(r * 32, 32)],
                                      sem_w.at[0]).start(priority=0)
                pltpu.make_async_copy(bx.at[b, pl.ds(r * 32, 32)], xbuf.at[1, b, pl.ds(r * 32, 32)],
                                      sem_w.at[0]).start(priority=1)
            return c
        lax.fori_loop(0, B, xloop, 0)

        def wloop(i, c):
            for cc in range(4):
                for half in range(2):
                    rq = pl.multiple_of(i * 16 + half * 256, 16)
                    ro = pl.multiple_of(i * 128 + cc * 32 + half * 2048, 32)
                    for br, (wq, wo) in enumerate(((awq, awo), (bwq, bwo))):
                        pltpu.make_async_copy(
                            wq.at[pl.ds(rq, 16), pl.ds(cc * 1024, 1024)],
                            wqbuf.at[br, pl.ds(rq, 16), pl.ds(cc * 1024, 1024)],
                            sem_w.at[1]).start(priority=0)
                        pltpu.make_async_copy(
                            wo.at[pl.ds(ro, 32)], wobuf.at[br, pl.ds(ro, 32)],
                            sem_w.at[2]).start(priority=1)
            return c
        lax.fori_loop(0, 16, wloop, 0)

        issue_unit(-1, only=1)
        for j in range(dist):
            issue_unit(j)
        pltpu.make_async_copy(xbuf, xbuf, sem_w.at[0]).wait()
        pltpu.make_async_copy(wqbuf, wqbuf, sem_w.at[1]).wait()
        pltpu.make_async_copy(wobuf, wobuf, sem_w.at[2]).wait()

        def out_copy(b):
            return pltpu.make_async_copy(obuf.at[b % 2], o_hbm.at[b], sem_o.at[b % 2])

        def step(j, do_prefetch):
            b, h = bh(j)

            @pl.when(j % H == 0)
            def _():
                acc[...] = jnp.zeros_like(acc)

            wait_kv(j)
            slot = j % nslot
            col = pl.multiple_of(h * Dh, Dh)
            qs = []
            for br in range(2):
                q = jnp.dot(xbuf[br, b], wqbuf[br, :, pl.ds(col, Dh)],
                            preferred_element_type=jnp.float32)
                qs.append((q * qscale).astype(jnp.bfloat16))

            def qk(br):
                return lax.dot_general(qs[br], kvbuf[slot, 2 * br], (((1,), (1,)), ((), ())),
                                       preferred_element_type=jnp.float32)

            def pv(br, s):
                m = jnp.max(s, axis=-1, keepdims=True)
                e = jnp.exp2(s - m)
                l = jnp.sum(e, axis=-1, keepdims=True)
                o = jnp.dot(e.astype(jnp.bfloat16), kvbuf[slot, 2 * br + 1],
                            preferred_element_type=jnp.float32)
                return (o * (1.0 / l)).astype(jnp.bfloat16)

            def oproj(br, o):
                acc[:, br * D:(br + 1) * D] += jnp.dot(
                    o, wobuf[br, pl.ds(col, Dh), :], preferred_element_type=jnp.float32)

            def pre(k):
                if do_prefetch:
                    for part in range(k * nparts // 2, (k + 1) * nparts // 2):
                        issue_unit(j + dist, part)

            s0 = qk(0)
            pre(0)
            s1 = qk(1)
            o0 = pv(0, s0)
            pre(1)
            o1 = pv(1, s1)
            oproj(0, o0)
            oproj(1, o1)

            @pl.when(j % H == H - 1)
            def _():
                @pl.when(b >= 2)
                def _():
                    out_copy(b - 2).wait()
                obuf[b % 2] = acc[...].astype(obuf.dtype)
                out_copy(b).start()

        def body_main(j, carry):
            step(j, True)
            return carry

        def body_tail(j, carry):
            step(j, False)
            return carry

        lax.fori_loop(0, NP - dist - 1, body_main, 0)
        issue_unit(NP - 1, only=0)
        lax.fori_loop(NP - dist - 1, NP, body_tail, 0)
        out_copy(B - 2).wait()
        out_copy(B - 1).wait()

    return pl.pallas_call(
        kern,
        in_specs=[pl.BlockSpec(memory_space=pl.ANY)] * 10,
        out_specs=pl.BlockSpec(memory_space=pl.ANY),
        out_shape=jax.ShapeDtypeStruct((B, Sq, 2 * D), jnp.bfloat16),
        scratch_shapes=[
            pltpu.VMEM((2, B, Sq, D), jnp.bfloat16),
            pltpu.VMEM((2, D, H * Dh), jnp.bfloat16),
            pltpu.VMEM((2, H * Dh, D), jnp.bfloat16),
            pltpu.VMEM((nslot, 4, Sk, Dh), jnp.bfloat16),
            pltpu.VMEM((Sq, 2 * D), jnp.float32),
            pltpu.VMEM((2, Sq, 2 * D), jnp.bfloat16),
            pltpu.SemaphoreType.DMA((3,)),
            pltpu.SemaphoreType.DMA((nslot,)),
            pltpu.SemaphoreType.DMA((2,)),
        ],
        compiler_params=pltpu.CompilerParams(
            vmem_limit_bytes=64 * 1024 * 1024, disable_bounds_checks=True),
    )(A_x, A_k_cache, A_v_cache, A_wq, A_wo, B_x, B_k_cache, B_v_cache, B_wq, B_wo)
```

```python
import jax
import jax.numpy as jnp
from jax import lax
from jax.experimental import pallas as pl
from jax.experimental.pallas import tpu as pltpu

_LOG2E = 1.4426950408889634

_R = 128
_NSLOT = 8
_DIST = 4
_OROWS = 16


@jax.jit
def pallas_concat_heads__mha_block_cached__gqa_block_cached__near_ridge_kernel(
    A_x: jax.Array,
    A_k_cache: jax.Array,
    A_v_cache: jax.Array,
    A_wq: jax.Array,
    A_wo: jax.Array,
    B_x: jax.Array,
    B_k_cache: jax.Array,
    B_v_cache: jax.Array,
    B_wq: jax.Array,
    B_wo: jax.Array,
):
    B, Sq, D = A_x.shape
    _, H, Sk, Dh = A_k_cache.shape
    assert B_k_cache.shape == A_k_cache.shape and B_v_cache.shape == A_v_cache.shape
    assert (B, Sq, D, H, Sk, Dh) == (8, 128, 512, 32, 1024, 128)
    R, nslot, dist = _R, _NSLOT, _DIST
    assert nslot >= dist + 2
    NP = B * H
    hc = (Sk // R) // 2
    hstride = H // 2
    qscale = Dh ** -0.5 * _LOG2E

    def bh(j):
        b = j // H
        t = j % H
        return b, (t % 2) * hstride + t // 2

    def kern(ax, ak, av, awq, awo, bx, bk, bv, bwq, bwo, o_hbm,
             xbuf, wqbuf, wobuf, kvbuf, acc, obuf, sem_w, sem_kv, sem_o):
        kv_src = (ak, av, bk, bv)

        def chunk_copy(j, c, a):
            b, h = bh(j)
            slot = j % nslot
            return pltpu.make_async_copy(
                kv_src[a].at[b, h, pl.ds(c * R, R)],
                kvbuf.at[slot, a, pl.ds(c * R, R)],
                sem_kv.at[slot])

        unit = [(dj, cc, a) for c in range(hc)
                for dj, cc in ((0, hc + c), (1, c)) for a in range(4)]

        def issue_unit(j, part=None, only=None):
            lst = unit
            if part is not None:
                per = len(lst) // 2
                lst = lst[part * per:(part + 1) * per]
            for dj, c, a in lst:
                if only is None or dj == only:
                    chunk_copy(j + dj, c, a).start(priority=a % 2)

        def wait_kv(j):
            slot = j % nslot
            pltpu.make_async_copy(kvbuf.at[slot], kvbuf.at[slot], sem_kv.at[slot]).wait()

        def out_start(bs):
            i = 0
            for c in range(Sq // _OROWS):
                for b in bs:
                    pltpu.make_async_copy(
                        obuf.at[b, pl.ds(c * _OROWS, _OROWS)],
                        o_hbm.at[b, pl.ds(c * _OROWS, _OROWS)],
                        sem_o.at[0]).start(priority=i % 2)
                    i += 1

        def xloop(b, c):
            for r in range(4):
                pltpu.make_async_copy(ax.at[b, pl.ds(r * 32, 32)], xbuf.at[0, b, pl.ds(r * 32, 32)],
                                      sem_w.at[0]).start(priority=0)
                pltpu.make_async_copy(bx.at[b, pl.ds(r * 32, 32)], xbuf.at[1, b, pl.ds(r * 32, 32)],
                                      sem_w.at[0]).start(priority=1)
            return c
        lax.fori_loop(0, B, xloop, 0)

        def wloop(i, c):
            for cc in range(4):
                for half in range(2):
                    rq = pl.multiple_of(i * 16 + (cc // 2) * 8 + half * 256, 8)
                    cq = (cc % 2) * 2048
                    ro = pl.multiple_of(i * 128 + cc * 32 + half * 2048, 32)
                    for br, (wq, wo) in enumerate(((awq, awo), (bwq, bwo))):
                        pltpu.make_async_copy(
                            wq.at[pl.ds(rq, 8), pl.ds(cq, 2048)],
                            wqbuf.at[br, pl.ds(rq, 8), pl.ds(cq, 2048)],
                            sem_w.at[1]).start(priority=0)
                        pltpu.make_async_copy(
                            wo.at[pl.ds(ro, 32)], wobuf.at[br, pl.ds(ro, 32)],
                            sem_w.at[2]).start(priority=1)
            return c
        lax.fori_loop(0, 16, wloop, 0)

        issue_unit(-1, only=1)
        for j in range(dist):
            issue_unit(j)
        pltpu.make_async_copy(xbuf, xbuf, sem_w.at[0]).wait()
        pltpu.make_async_copy(wqbuf, wqbuf, sem_w.at[1]).wait()
        pltpu.make_async_copy(wobuf, wobuf, sem_w.at[2]).wait()

        def step(j, prefetch):
            b, h = bh(j)

            @pl.when(j % H == 0)
            def _():
                acc[...] = jnp.zeros_like(acc)

            if not prefetch:
                @pl.when(j == NP - 2)
                def _():
                    out_start(range(B - 1))

            wait_kv(j)
            slot = j % nslot
            col = pl.multiple_of(h * Dh, Dh)
            if prefetch:
                issue_unit(j + dist, part=0)

            qs = []
            for br in range(2):
                q = jnp.dot(xbuf[br, b], wqbuf[br, :, pl.ds(col, Dh)],
                            preferred_element_type=jnp.float32)
                qs.append((q * qscale).astype(jnp.bfloat16))

            def qk(br):
                return lax.dot_general(qs[br], kvbuf[slot, 2 * br], (((1,), (1,)), ((), ())),
                                       preferred_element_type=jnp.float32)

            def pv(br, s):
                m = jnp.max(s, axis=-1, keepdims=True)
                e = jnp.exp2(s - m)
                l = jnp.sum(e, axis=-1, keepdims=True)
                o = jnp.dot(e.astype(jnp.bfloat16), kvbuf[slot, 2 * br + 1],
                            preferred_element_type=jnp.float32)
                return (o * (1.0 / l)).astype(jnp.bfloat16)

            def oproj(br, o):
                acc[:, br * D:(br + 1) * D] += jnp.dot(
                    o, wobuf[br, pl.ds(col, Dh), :], preferred_element_type=jnp.float32)

            s0 = qk(0)
            s1 = qk(1)
            o0 = pv(0, s0)
            o1 = pv(1, s1)
            if prefetch:
                issue_unit(j + dist, part=1)
            oproj(0, o0)
            oproj(1, o1)

            @pl.when(j % H == H - 1)
            def _():
                obuf[b] = acc[...].astype(obuf.dtype)

        def body_main(j, carry):
            step(j, True)
            return carry

        def body_tail(j, carry):
            step(j, False)
            return carry

        lax.fori_loop(0, NP - dist - 1, body_main, 0)
        issue_unit(NP - 1, only=0)
        lax.fori_loop(NP - dist - 1, NP, body_tail, 0)
        out_start([B - 1])
        pltpu.make_async_copy(obuf, o_hbm, sem_o.at[0]).wait()

    return pl.pallas_call(
        kern,
        in_specs=[pl.BlockSpec(memory_space=pl.ANY)] * 10,
        out_specs=pl.BlockSpec(memory_space=pl.ANY),
        out_shape=jax.ShapeDtypeStruct((B, Sq, 2 * D), jnp.bfloat16),
        scratch_shapes=[
            pltpu.VMEM((2, B, Sq, D), jnp.bfloat16),
            pltpu.VMEM((2, D, H * Dh), jnp.bfloat16),
            pltpu.VMEM((2, H * Dh, D), jnp.bfloat16),
            pltpu.VMEM((nslot, 4, Sk, Dh), jnp.bfloat16),
            pltpu.VMEM((Sq, 2 * D), jnp.float32),
            pltpu.VMEM((B, Sq, 2 * D), jnp.bfloat16),
            pltpu.SemaphoreType.DMA((3,)),
            pltpu.SemaphoreType.DMA((nslot,)),
            pltpu.SemaphoreType.DMA((1,)),
        ],
        compiler_params=pltpu.CompilerParams(
            vmem_limit_bytes=64 * 1024 * 1024, disable_bounds_checks=True),
    )(A_x, A_k_cache, A_v_cache, A_wq, A_wo, B_x, B_k_cache, B_v_cache, B_wq, B_wo)
```
